```python
import os as _os
_os.environ.setdefault("JAX_PLATFORMS", "cpu")
import jax
import jax.numpy as jnp

def _softmax(x, axis=-1):
    return jax.nn.softmax(x, axis=axis)
def _gelu(x):
    return jax.nn.gelu(x, approximate=True)
def _silu(x):
    return jax.nn.silu(x)
def _sigmoid(x):
    return jax.nn.sigmoid(x)
def _layernorm(x, axis=-1, eps=1e-5):
    m = jnp.mean(x, axis=axis, keepdims=True)
    v = jnp.var(x, axis=axis, keepdims=True)
    return (x - m) / jnp.sqrt(v + eps)
def _scatter_add(tgt, idx, src, axis=0):
    return tgt.at[idx].add(src)
def _segment_sum(src, seg, n):
    return jax.ops.segment_sum(src, seg, n)
class _Rng:
    def __init__(self, key):
        self._k = key
    def _next(self):
        self._k, sub = jax.random.split(self._k)
        return sub
    def normal(self, shape):
        return jax.random.normal(self._next(), shape, dtype=jnp.bfloat16)
    def randint(self, lo, hi, shape):
        return jax.random.randint(self._next(), shape, lo, hi, dtype=jnp.int32)
    def uniform(self, shape, lo=0.0, hi=1.0):
        return jax.random.uniform(self._next(), shape, jnp.bfloat16, lo, hi)
    def permutation(self, n):
        return jax.random.permutation(self._next(), n)


kernel_name = 'parallel_sum__sliding_local_dilated__glu_gated_geglu__prompt'

def setup_inputs():
    _rng = _Rng(jax.random.key(int.from_bytes(__import__("os").urandom(4), "little")))
    _w = (lambda a: (lambda t: t.astype(jnp.bfloat16) if jnp.issubdtype(t.dtype, jnp.floating) else t)(jnp.asarray(a)))
    def _A_setup():
        B, S, D = 1, 2048, 512
        return {
            "x": _w((lambda *s: _rng.normal(s) * 0.05)(B, S, D)),
            "wqkv": _w((lambda *s: _rng.normal(s) * 0.05)(D, 3 * D)),
            "wo": _w((lambda *s: _rng.normal(s) * 0.05)(D, D)),
        }
    _A_in = _A_setup()

    def _B_setup():
        B, S, Dm, Df = 1, 2048, 512, 1376
        return {
            "x": _w((lambda *s: _rng.normal(s) * 0.05)(B, S, Dm)),
            "w_gate": _w((lambda *s: _rng.normal(s) * 0.1)(Dm, Df) * (Dm ** -0.5)),
            "w_up": _w((lambda *s: _rng.normal(s) * 0.1)(Dm, Df) * (Dm ** -0.5)),
            "w_down": _w((lambda *s: _rng.normal(s) * 0.1)(Df, Dm) * (Df ** -0.5)),
        }
    _B_in = _B_setup()

    return {
        "A_x": _A_in["x"],
        "A_wqkv": _A_in["wqkv"],
        "A_wo": _A_in["wo"],
        "B_x": _B_in["x"],
        "B_w_gate": _B_in["w_gate"],
        "B_w_up": _B_in["w_up"],
        "B_w_down": _B_in["w_down"],
    }

def reference(A_x, A_wqkv, A_wo, B_x, B_w_gate, B_w_up, B_w_down):
    def _A_ref(x, wqkv, wo):
        B, S, D = x.shape
        H = 32; Dh = D // H
        W, dil = 8, 2
        qkv = (lambda x, *d: x.transpose(*d))((x @ wqkv).reshape(B, S, 3, H, Dh), 2, 0, 3, 1, 4)
        q, k, v = qkv[0], qkv[1], qkv[2]
        scale = Dh ** -0.5
        pos = jnp.arange(S)
        off = jnp.arange(W) * dil
        idx = pos[:, None] - off[None, :]
        mask = idx >= 0
        idx_c = jnp.where(mask, idx, 0).reshape(-1)
        kg = k[:, :, idx_c, :].reshape(B, H, S, W, Dh)
        vg = v[:, :, idx_c, :].reshape(B, H, S, W, Dh)
        logits = jnp.einsum("bhsd,bhswd->bhsw", q, kg) * scale
        logits = jnp.where(mask[None, None, :, :], logits, -1e9)
        attn = _softmax(logits, axis=-1)
        o = jnp.einsum("bhsw,bhswd->bhsd", attn, vg)
        return (lambda x, *d: x.transpose(*d))(o, 0, 2, 1, 3).reshape(B, S, D) @ wo

    def _B_ref(x, w_gate, w_up, w_down):
        g = jnp.einsum("bsd,df->bsf", x, w_gate)
        u = jnp.einsum("bsd,df->bsf", x, w_up)
        h = _gelu(g) * u
        return jnp.einsum("bsf,fd->bsd", h, w_down)

    x = A_x
    xn = _layernorm(x, axis=-1)
    return x + _A_ref(xn, A_wqkv, A_wo) + _B_ref(xn, B_w_gate, B_w_up, B_w_down)
```

```python
import functools
import contextlib
import numpy as np
import jax
import jax.numpy as jnp
from jax import lax
import jax.experimental.pallas as pl
import jax.experimental.pallas.tpu as pltpu

S, D, F = 2048, 512, 1376
H, DH, W, DIL = 32, 16, 8, 2
HALO = 16
TM = 256
NB = S // TM
RB = 8
LOG2E = float(np.log2(np.e))
QS = (DH ** -0.5) * LOG2E
C1 = float(np.sqrt(2.0 / np.pi))
C2 = C1 * 0.044715
NT = (((1,), (1,)), ((), ()))
f32, bf16, u32 = jnp.float32, jnp.bfloat16, jnp.uint32
FLAGS = None
SCOPES = 0
scope = (lambda n: jax.named_scope(n)) if SCOPES else (lambda n: contextlib.nullcontext())
P = {}

WCH = P.get("wch", [(0, 128), (128, 384), (384, 896), (896, 1376)])
FCH = P.get("fch", [(0, 256), (256, 512), (512, 768), (768, 1024), (1024, 1376)])
DMAS = [("x", 0, 256), ("x", 256, 256), ("g", 0), ("u", 0), ("g", 1), ("u", 1), ("g", 2), ("u", 2), ("g", 3), ("u", 3),
        ("x", 512, 256), ("qkv",), ("x", 768, 1280), ("wo",), ("wd",)]
NDMA = len(DMAS)


def _body(x_hbm, wqkv_hbm, wo_hbm, wg_hbm, wu_hbm, wd_hbm, out_hbm,
          x_v, wqkv_v, wqkvp_v, wo_v, wop_v, wop_t, wg_v, wu_v, wd_v, out_v,
          xn_s, q_s, k_s, v_s, ob_s, h_s, pw_s, sems, sem_o):

    def dma(i):
        d = DMAS[i]
        if d[0] == "x":
            return pltpu.make_async_copy(x_hbm.at[0, pl.ds(d[1], d[2]), :], x_v.at[pl.ds(d[1], d[2]), :], sems.at[i])
        if d[0] in ("g", "u"):
            a, e = WCH[d[1]]
            src, dst = (wg_hbm, wg_v) if d[0] == "g" else (wu_hbm, wu_v)
            return pltpu.make_async_copy(src.at[pl.ds(a, e - a), :], dst.at[pl.ds(a, e - a), :], sems.at[i])
        src, dst = {"qkv": (wqkv_hbm, wqkv_v), "wo": (wo_hbm, wo_v), "wd": (wd_hbm, wd_v)}[d[0]]
        return pltpu.make_async_copy(src, dst, sems.at[i])

    def wait(*names):
        for i, d in enumerate(DMAS):
            if d in names or d[:2] in names:
                dma(i).wait()

    def cp_out(b):
        return pltpu.make_async_copy(out_v.at[pl.ds(b * TM, TM), :], out_hbm.at[0, pl.ds(b * TM, TM), :], sem_o.at[b])

    for i in range(NDMA):
        dma(i).start()

    def ln(b):
        r = pl.ds(b * TM, TM)
        x = x_v[r, :].astype(f32)
        m = jnp.mean(x, axis=-1, keepdims=True)
        xc = x - m
        var = jnp.mean(xc * xc, axis=-1, keepdims=True)
        xn_s[r, :] = (xc * lax.rsqrt(var + 1e-5)).astype(bf16)

    def gate(b, a, e, groups=()):
        r = pl.ds(b * TM, TM)
        xn = xn_s[r, :]
        g = lax.dot_general(xn, wg_v[a:e, :], NT, preferred_element_type=f32)
        u = lax.dot_general(xn, wu_v[a:e, :], NT, preferred_element_type=f32)
        t = jnp.tanh(g * (C1 + C2 * (g * g)))
        hu = (0.5 * g) * u
        h_s[r, a:e] = (hu + hu * t).astype(bf16)
        n = len(groups)
        nfull = (e - a) // 128
        for i, r0 in enumerate(groups):
            pos = (i * nfull * (TM // 8)) // n
            tile, row = pos // (TM // 8), pos % (TM // 8)
            attn(r0, u[row * 8:(row + 1) * 8, tile * 128:(tile + 1) * 128])

    def prep_qkv():
        lane = lax.broadcasted_iota(jnp.int32, (8, 128), 1)
        src = (lane & 7) * 16 + ((lane >> 3) & 3) * 4 + (lane >> 5)
        tgt = wqkvp_v.bitcast(u32)
        srcr = wqkv_v.bitcast(u32)
        for r0 in range(0, D // 2, 8):
            for c in range(12):
                pw_s[r0:r0 + 8, c * 128:(c + 1) * 128] = jnp.take_along_axis(srcr[r0:r0 + 8, c * 128:(c + 1) * 128], src, axis=1)
        for bit, pairs, last in ((8, ((0, 1), (2, 3)), False), (16, ((0, 2), (1, 3)), True)):
            msk = (lane & bit) != 0
            dst = tgt if last else pw_s
            for r0 in range(0, D // 2, 8):
                for mtx in range(3):
                    for (ia, ib) in pairs:
                        ca, cb = (mtx * 4 + ia) * 128, (mtx * 4 + ib) * 128
                        a = pw_s[r0:r0 + 8, ca:ca + 128]
                        bb = pw_s[r0:r0 + 8, cb:cb + 128]
                        p = jnp.take_along_axis(jnp.where(msk, a, bb), lane ^ bit, axis=1)
                        dst[r0:r0 + 8, ca:ca + 128] = jnp.where(msk, p, a)
                        dst[r0:r0 + 8, cb:cb + 128] = jnp.where(msk, bb, p)

    def prep_wo():
        for c in range(4):
            for h in range(H):
                wop_t[c, h * 17:h * 17 + 16, :] = wo_v[h * 16:(h + 1) * 16, c * 128:(c + 1) * 128].astype(f32)
        for c in range(4):
            for d in range(DH):
                wop_v[d * 32:(d + 1) * 32, c * 128:(c + 1) * 128] = wop_t[c, pl.ds(d, H, stride=17), :].astype(bf16)

    def qkv(b):
        r = pl.ds(b * TM, TM)
        rk = pl.ds(HALO + b * TM, TM)
        xn = xn_s[r, :]
        for c in range(4):
            k_s[c, rk, :] = jnp.dot(xn, wqkvp_v[:, D + c * 128:D + (c + 1) * 128], preferred_element_type=f32)
        for c in range(4):
            q_s[c, r, :] = jnp.dot(xn, wqkvp_v[:, c * 128:(c + 1) * 128], preferred_element_type=f32)
        for c in range(4):
            v_s[c, rk, :] = jnp.dot(xn, wqkvp_v[:, 2 * D + c * 128:2 * D + (c + 1) * 128], preferred_element_type=f32)

    def attn(r0, dep=None):
        q = [q_s[c, r0:r0 + RB, :] for c in range(4)]
        if dep is not None:
            z = pltpu.bitcast(pltpu.bitcast(dep, u32) & jnp.uint32(0x80000000), f32)
            scl = z + QS
            q = [t * scl for t in q]
        else:
            q = [t * QS for t in q]
        lg = []
        for w in range(W):
            st = HALO + r0 - DIL * w
            p = [q[c] * k_s[c, st:st + RB, :] for c in range(4)]
            a = (p[0] + p[1]) + (p[2] + p[3])
            a = a + pltpu.roll(a, 64, 1)
            a = a + pltpu.roll(a, 32, 1)
            if r0 < DIL * (W - 1) and w > 0:
                row = r0 + lax.broadcasted_iota(jnp.int32, (RB, 128), 0)
                a = jnp.where(row >= DIL * w, a, -1e9 * LOG2E)
            lg.append(a)
        mx = functools.reduce(jnp.maximum, lg)
        e = [jnp.exp2(a - mx) for a in lg]
        den = functools.reduce(lambda a, b: a + b, e)
        inv = pl.reciprocal(den, approx=True)
        inv = inv * (2.0 - den * inv)
        for c in range(4):
            acc = None
            for w in range(W):
                st = HALO + r0 - DIL * w
                t = e[w] * v_s[c, st:st + RB, :]
                acc = t if acc is None else acc + t
            ob_s[r0:r0 + RB, c * 128:(c + 1) * 128] = (acc * inv).astype(bf16)

    def down(b):
        r = pl.ds(b * TM, TM)
        y = jnp.dot(h_s[r, :], wd_v[...], preferred_element_type=f32)
        y = y + jnp.dot(ob_s[r, :], wop_v[...], preferred_element_type=f32)
        out_v[r, :] = (y + x_v[r, :].astype(f32)).astype(bf16)
        cp_out(b).start()

    z = jnp.zeros((4, HALO, 128), f32)
    k_s[:, 0:HALO, :] = z
    v_s[:, 0:HALO, :] = z

    with scope("p0"):
        wait(("x", 0))
        ln(0)
        wait(("x", 256), ("g", 0), ("u", 0))
        ln(1)
    for j in range(len(WCH)):
        with scope(f"p1_{j}"):
            if j > 0:
                wait(("g", j), ("u", j))
            if j == len(WCH) - 1:
                wait(("x", 512))
            for b in range(2):
                gate(b, *WCH[j])
    ln(2)
    with scope("p2_g2"):
        for (a, e) in FCH:
            gate(2, a, e)
    with scope("p3_wait"):
        wait(("qkv",), ("x", 768), ("wo",), ("wd",))
    with scope("p4_g3prep"):
        prep_qkv()
        for b in range(3, NB):
            ln(b)
        for (a, e) in FCH:
            gate(3, a, e)
        prep_wo()
    with scope("p5_q"):
        for b in range(NB):
            qkv(b)
    groups = list(range(0, S, RB))
    slots = [(b, a, e) for b in range(4, NB) for (a, e) in FCH]
    tot = sum((e - a) // 128 for (_, a, e) in slots)
    NA = P.get("NA", len(groups))
    acc, gi = 0, 0
    for (b, a, e) in slots:
        acc += (e - a) // 128
        ge = (NA * acc) // tot
        with scope(f"p6_ga{b}"):
            gate(b, a, e, groups[gi:ge])
        gi = ge
    for r0 in groups[gi:]:
        attn(r0)
    for b in range(NB):
        with scope(f"p7_d{b}"):
            down(b)
    for b in range(NB):
        cp_out(b).wait()


@jax.jit
def pallas_parallel_sum__sliding_local_dilated__glu_gated_geglu__prompt_kernel(A_x, A_wqkv, A_wo, B_x, B_w_gate, B_w_up, B_w_down):
    anyspec = pl.BlockSpec(memory_space=pl.ANY)
    V = pltpu.VMEM
    return pl.pallas_call(
        _body,
        in_specs=[anyspec] * 6,
        out_specs=anyspec,
        out_shape=jax.ShapeDtypeStruct((1, S, D), bf16),
        scratch_shapes=[
            V((S, D), bf16), V((D, 3 * D), bf16), V((D, 3 * D), bf16), V((D, D), bf16), V((D, D), bf16),
            V((4, H * 17, 128), f32),
            V((F, D), bf16), V((F, D), bf16), V((F, D), bf16), V((S, D), bf16),
            V((S, D), bf16), V((4, S, 128), f32), V((4, HALO + S, 128), f32), V((4, HALO + S, 128), f32),
            V((S, D), bf16), V((S, F), bf16), V((D // 2, 3 * D), u32),
            pltpu.SemaphoreType.DMA((NDMA,)), pltpu.SemaphoreType.DMA((NB,)),
        ],
        compiler_params=pltpu.CompilerParams(vmem_limit_bytes=100 * 2**20, flags=FLAGS),
        name="fused",
    )(A_x, A_wqkv, A_wo, B_w_gate.T, B_w_up.T, B_w_down)
```

```python
import functools

import numpy as np
import jax
import jax.numpy as jnp
from jax import lax
import jax.experimental.pallas as pl
import jax.experimental.pallas.tpu as pltpu

S, D, F = 2048, 512, 1376
H, DH, W, DIL = 32, 16, 8, 2
HALO = 16
RB = 8
LOG2E = float(np.log2(np.e))
QS = (DH ** -0.5) * LOG2E
C1 = float(np.sqrt(2.0 / np.pi))
C2 = C1 * 0.044715
NT = (((1,), (1,)), ((), ()))
f32, bf16, u32 = jnp.float32, jnp.bfloat16, jnp.uint32

MG = 256
MQ = 256
DSZ = (512, 512, 512, 256, 256)
FREM = 1280
WCH = ((0, 128), (128, 256), (256, 512), (512, 896), (896, F))
FCH = ((0, 256), (256, 512), (512, 768), (768, 1024), (1024, FREM))
DMAS = [("x", 0, 256), ("g", 0), ("u", 0), ("x", 256, 128), ("x", 384, 128)]
for _j in range(1, len(WCH)):
    DMAS += [("g", _j), ("u", _j)]
DMAS += [("x", 512, 512), ("qkv",), ("x", 1024, 1024), ("wo",), ("wd",)]
NDMA = len(DMAS)
NPACE = len(WCH) + 3


def _body(x_hbm, wqkv_hbm, wo_hbm, wg_hbm, wu_hbm, wd_hbm, out_hbm,
          x_v, wqkv_v, wqkvp_v, wo_v, wop_v, wop_t, wg_v, wu_v, wd_v, out_v,
          xn_s, q_s, k_s, v_s, ob_s, h_s, pw_s, dum, sems, sem_o):

    def dma(i):
        d = DMAS[i]
        if d[0] == "x":
            return pltpu.make_async_copy(
                x_hbm.at[0, pl.ds(d[1], d[2]), :], x_v.at[pl.ds(d[1], d[2]), :], sems.at[i])
        if d[0] in ("g", "u"):
            a, e = WCH[d[1]]
            src, dst = (wg_hbm, wg_v) if d[0] == "g" else (wu_hbm, wu_v)
            return pltpu.make_async_copy(
                src.at[pl.ds(a, e - a), :], dst.at[pl.ds(a, e - a), :], sems.at[i])
        src, dst = {"qkv": (wqkv_hbm, wqkv_v), "wo": (wo_hbm, wo_v), "wd": (wd_hbm, wd_v)}[d[0]]
        return pltpu.make_async_copy(src, dst, sems.at[i])

    def wait(*names):
        for i, d in enumerate(DMAS):
            if d in names or d[:2] in names:
                dma(i).wait()

    def cp_out(r0, n, c0=0, nc=D):
        return pltpu.make_async_copy(
            out_v.at[pl.ds(r0, n), pl.ds(c0, nc)],
            out_hbm.at[0, pl.ds(r0, n), pl.ds(c0, nc)], sem_o.at[0])

    for i in range(NDMA):
        dma(i).start()

    paces = []

    def pace(val, back):
        k = len(paces)
        n = val.shape[0]
        dum[k] = val[n - back:n - back + 16, val.shape[1] - 128:]
        c = pltpu.make_async_copy(
            x_hbm.at[0, pl.ds(0, 16), pl.ds(0, 128)], dum.at[k], sems.at[NDMA + k])
        c.start()
        paces.append(c)

    def ld(ref, r0, n, c0=None, c1=None):
        c = slice(None) if c0 is None else slice(c0, c1)
        return pltpu.bitcast(ref[r0 // 2:(r0 + n) // 2, c], bf16)

    def st(ref, r0, val, c0=None, c1=None):
        c = slice(None) if c0 is None else slice(c0, c1)
        ref[r0 // 2:(r0 + val.shape[0]) // 2, c] = pltpu.bitcast(val, u32)

    def ln(r0, n=256):
        x = x_v[r0:r0 + n, :].astype(f32)
        m = jnp.mean(x, axis=-1, keepdims=True)
        xc = x - m
        var = jnp.mean(xc * xc, axis=-1, keepdims=True)
        rs = lax.rsqrt(var + 1e-5)
        st(xn_s, r0, (xc * rs).astype(bf16))
        return rs

    def geglu(g, u):
        t = jnp.tanh(g * (C1 + C2 * (g * g)))
        hu = (0.5 * g) * u
        return hu + hu * t

    def gate(r0, n, a, e, groups=()):
        xn = ld(xn_s, r0, n)
        g = lax.dot_general(xn, wg_v[a:e, :], NT, preferred_element_type=f32)
        u = lax.dot_general(xn, wu_v[a:e, :], NT, preferred_element_type=f32)
        hv = geglu(g, u).astype(bf16)
        st(h_s, r0, hv, a, e)
        host([u[:, t * 128:(t + 1) * 128] for t in range((e - a) // 128)], groups)
        return g, hv

    def gate_rem(r0, n, groups=()):
        a, e = FREM, F
        xn = ld(xn_s, r0, n)
        wgu = jnp.concatenate([wg_v[a:e, :], wu_v[a:e, :]], axis=0)
        r = lax.dot_general(wgu, xn, NT, preferred_element_type=f32)
        st(h_s, r0, geglu(r[:e - a], r[e - a:]).T.astype(bf16), a, e)
        host([r[:, t * 128:(t + 1) * 128] for t in range(n // 128)], groups)

    def host(tiles, groups):
        n = len(groups)
        per = tiles[0].shape[0] // RB
        for i, r0 in enumerate(groups):
            pos = ((2 * i + 1) * len(tiles) * per) // (2 * n)
            tile, row = pos // per, pos % per
            attn(r0, tiles[tile][row * RB:(row + 1) * RB, :])

    def prep_qkv():
        lane = lax.broadcasted_iota(jnp.int32, (8, 128), 1)
        src = (lane & 7) * 16 + ((lane >> 3) & 3) * 4 + (lane >> 5)
        for r0 in range(0, D // 2, 8):
            for c in range(12):
                pw_s[r0:r0 + 8, c * 128:(c + 1) * 128] = jnp.take_along_axis(
                    pltpu.bitcast(wqkv_v[2 * r0:2 * r0 + 16, c * 128:(c + 1) * 128], u32), src, axis=1)
        for bit, pairs, last in ((8, ((0, 1), (2, 3)), False), (16, ((0, 2), (1, 3)), True)):
            msk = (lane & bit) != 0
            dst = wqkvp_v if last else pw_s
            for r0 in range(0, D // 2, 8):
                for mtx in range(3):
                    for (ia, ib) in pairs:
                        ca, cb = (mtx * 4 + ia) * 128, (mtx * 4 + ib) * 128
                        a = pw_s[r0:r0 + 8, ca:ca + 128]
                        b = pw_s[r0:r0 + 8, cb:cb + 128]
                        p = jnp.take_along_axis(jnp.where(msk, a, b), lane ^ bit, axis=1)
                        dst[r0:r0 + 8, ca:ca + 128] = jnp.where(msk, p, a)
                        dst[r0:r0 + 8, cb:cb + 128] = jnp.where(msk, b, p)

    def prep_wo():
        for c in range(4):
            for h in range(H):
                wop_t[c, h * 17:h * 17 + 16, :] = wo_v[h * 16:(h + 1) * 16, c * 128:(c + 1) * 128].astype(f32)
        for c in range(4):
            for d in range(DH):
                st(wop_v, d * 32, wop_t[c, pl.ds(d, H, stride=17), :].astype(bf16), c * 128, (c + 1) * 128)

    def qkv(r0, n, groups=()):
        xn = ld(xn_s, r0, n)
        tiles = []
        for (ref, base, off) in ((k_s, D, HALO), (q_s, 0, 0), (v_s, 2 * D, HALO)):
            for c in range(4):
                t = jnp.dot(xn, ld(wqkvp_v, 0, D, base + c * 128, base + (c + 1) * 128),
                            preferred_element_type=f32)
                ref[c, off + r0:off + r0 + n, :] = t
                tiles.append(t)
        host(tiles, groups)

    def attn(r0, dep):
        z = pltpu.bitcast(pltpu.bitcast(dep, u32) & jnp.uint32(0x80000000), f32)
        scl = z + QS
        q = [q_s[c, r0:r0 + RB, :] * scl for c in range(4)]
        lg = []
        for w in range(W):
            s0 = HALO + r0 - DIL * w
            p = [q[c] * k_s[c, s0:s0 + RB, :] for c in range(4)]
            a = (p[0] + p[1]) + (p[2] + p[3])
            a = a + pltpu.roll(a, 64, 1)
            a = a + pltpu.roll(a, 32, 1)
            if r0 < DIL * (W - 1) and w > 0:
                row = r0 + lax.broadcasted_iota(jnp.int32, (RB, 128), 0)
                a = jnp.where(row >= DIL * w, a, -1e9 * LOG2E)
            lg.append(a)
        mx = functools.reduce(jnp.maximum, lg)
        e = [jnp.exp2(a - mx) for a in lg]
        den = functools.reduce(lambda a, b: a + b, e)
        inv = pl.reciprocal(den, approx=True)
        inv = inv * (2.0 - den * inv)
        for c in range(4):
            acc = None
            for w in range(W):
                s0 = HALO + r0 - DIL * w
                t = e[w] * v_s[c, s0:s0 + RB, :]
                acc = t if acc is None else acc + t
            ob_s[r0:r0 + RB, c * 128:(c + 1) * 128] = (acc * inv).astype(bf16)

    def down(r0, n, groups=()):
        yh = jnp.dot(ld(h_s, r0, n, 0, F), wd_v[...], preferred_element_type=f32)
        yo = jnp.dot(ob_s[r0:r0 + n, :], ld(wop_v, 0, D), preferred_element_type=f32)
        y = (yh + yo + x_v[r0:r0 + n, :].astype(f32)).astype(bf16)
        if r0 + n == S:
            for c in range(4):
                out_v[r0:r0 + n, c * 128:(c + 1) * 128] = y[:, c * 128:(c + 1) * 128]
                cp_out(r0, n, c * 128, 128).start()
        else:
            out_v[r0:r0 + n, :] = y
            cp_out(r0, n).start()
        host([yh[:, t * 128:(t + 1) * 128] for t in range(4)], groups)

    zero = jnp.zeros((4, HALO, 128), f32)
    k_s[:, 0:HALO, :] = zero
    v_s[:, 0:HALO, :] = zero

    wait(("x", 0))
    rs = ln(0)
    acc = rs[0:16]
    for i in range(16, 256, 16):
        acc = acc + rs[i:i + 16]
    pace(jnp.broadcast_to(acc, (16, 128)).astype(bf16), 16)
    wait(("g", 0), ("u", 0))
    g0, hv = gate(0, 256, *WCH[0])
    pace(g0.astype(bf16), 192)
    wait(("x", 256))
    ln(256, 128)
    pace(hv, 240)
    wait(("x", 384))
    ln(384, 128)
    _, hv = gate(256, 128, *WCH[0])
    gate(384, 128, *WCH[0])
    for j in range(1, len(WCH)):
        pace(hv, 64 if j == 1 else 224)
        wait(("g", j), ("u", j))
        if j == len(WCH) - 1:
            wait(("x", 512))
            for r0 in (0, 256):
                gate_rem(r0, 256)
        for r0 in (0, 256):
            _, hv = gate(r0, 256, WCH[j][0], min(WCH[j][1], FREM))
    ln(512)
    ln(768)

    calls = []
    for r0 in range(512, 1024, MG):
        calls.append((r0, None))
        calls += [(r0, ch) for ch in FCH]
    npre = len(calls) // 2
    for i, (r0, ch) in enumerate(calls):
        if i == npre:
            pace(hv, 224)
            wait(("qkv",), ("x", 1024), ("wo",), ("wd",))
            prep_qkv()
        if npre <= i < npre + 4:
            ln(1024 + (i - npre) * 256)
        if ch is None:
            gate_rem(r0, MG)
        else:
            _, hv = gate(r0, MG, *ch)
    prep_wo()

    hosts = []
    for r0 in range(0, S, MQ):
        hosts.append((12 * MQ, ("q", r0, MQ)))
    for r0 in range(1024, S, MG):
        hosts.append((MG + MG // 2, ("r", r0, MG)))
        for (a, e) in FCH:
            hosts.append((((e - a) // 128) * 2 * MG, ("g", r0, MG, a, e)))
    r0 = 0
    for n in DSZ:
        hosts.append((15 * n, ("d", r0, n)))
        r0 += n
    t_first = 12 * MQ
    t_last = sum(d for d, _ in hosts) - 15 * DSZ[-1]
    groups = list(range(0, S, RB))
    ng = len(groups)
    t, gi = 0, 0
    for d, hd in hosts:
        t += d
        ge = max(gi, min(ng, (ng * (t - t_first)) // (t_last - t_first)))
        gs = groups[gi:ge]
        if hd[0] == "q":
            gs = [g for g in gs if g < hd[1]]
        if hd[0] == "d":
            assert gi == ng or groups[gi] >= hd[1] + hd[2]
        gi += len(gs)
        if hd[0] == "q":
            qkv(hd[1], hd[2], gs)
        elif hd[0] == "r":
            gate_rem(hd[1], hd[2], gs)
        elif hd[0] == "g":
            gate(hd[1], hd[2], hd[3], hd[4], gs)
        else:
            down(hd[1], hd[2], gs)
    assert gi == ng

    for c in paces:
        c.wait()
    pltpu.make_async_copy(out_v, out_hbm.at[0], sem_o.at[0]).wait()


@jax.jit
def pallas_parallel_sum__sliding_local_dilated__glu_gated_geglu__prompt_kernel(
    A_x: jax.Array,
    A_wqkv: jax.Array,
    A_wo: jax.Array,
    B_x: jax.Array,
    B_w_gate: jax.Array,
    B_w_up: jax.Array,
    B_w_down: jax.Array,
):
    del B_x
    hbm = pl.BlockSpec(memory_space=pl.ANY)
    V = pltpu.VMEM
    return pl.pallas_call(
        _body,
        in_specs=[hbm] * 6,
        out_specs=hbm,
        out_shape=jax.ShapeDtypeStruct((1, S, D), bf16),
        scratch_shapes=[
            V((S, D), bf16),
            V((D, 3 * D), bf16),
            V((D // 2, 3 * D), u32),
            V((D, D), bf16),
            V((D // 2, D), u32),
            V((4, H * 17, 128), f32),
            V((F, D), bf16),
            V((F, D), bf16),
            V((F, D), bf16),
            V((S, D), bf16),
            V((S // 2, D), u32),
            V((4, S, 128), f32),
            V((4, HALO + S, 128), f32),
            V((4, HALO + S, 128), f32),
            V((S, D), bf16),
            V((S // 2, F), u32),
            V((D // 2, 3 * D), u32),
            V((NPACE, 16, 128), bf16),
            pltpu.SemaphoreType.DMA((NDMA + NPACE,)),
            pltpu.SemaphoreType.DMA((1,)),
        ],
        compiler_params=pltpu.CompilerParams(
            vmem_limit_bytes=100 * 2**20,
            disable_semaphore_checks=True,
            flags={"XLA_TPU_RESCHEDULE_DMA_DONES": True},
        ),
        name="fused",
    )(A_x, A_wqkv, A_wo, B_w_gate.T, B_w_up.T, B_w_down)
```
